```python
import os as _os
_os.environ.setdefault('JAX_PLATFORMS', 'cpu')
import jax
import jax.numpy as jnp

def _softmax(x, axis=-1):
    return jax.nn.softmax(x, axis=axis)

def _gelu(x):
    return jax.nn.gelu(x, approximate=True)

def _silu(x):
    return jax.nn.silu(x)

def _sigmoid(x):
    return jax.nn.sigmoid(x)

def _layernorm(x, axis=-1, eps=1e-05):
    m = jnp.mean(x, axis=axis, keepdims=True)
    v = jnp.var(x, axis=axis, keepdims=True)
    return (x - m) / jnp.sqrt(v + eps)

def _scatter_add(tgt, idx, src, axis=0):
    return tgt.at[idx].add(src)

def _segment_sum(src, seg, n):
    return jax.ops.segment_sum(src, seg, n)

class _Rng:

    def __init__(self, key):
        self._k = key

    def _next(self):
        self._k, sub = jax.random.split(self._k)
        return sub

    def normal(self, shape):
        return jax.random.normal(self._next(), shape, dtype=jnp.bfloat16)

    def randint(self, lo, hi, shape):
        return jax.random.randint(self._next(), shape, lo, hi, dtype=jnp.int32)

    def uniform(self, shape, lo=0.0, hi=1.0):
        return jax.random.uniform(self._next(), shape, jnp.bfloat16, lo, hi)

    def permutation(self, n):
        return jax.random.permutation(self._next(), n)
kernel_name = 'adaLN_cond__linear_kernel_hedgehog__geglu_ffn__prompt'

def setup_inputs():
    _rng = _Rng(jax.random.key(int.from_bytes(__import__("os").urandom(4), "little")))
    _w = lambda a: (lambda t: t.astype(jnp.bfloat16) if jnp.issubdtype(t.dtype, jnp.floating) else t)(jnp.asarray(a))

    def _A_setup():
        B, S, D, H = (1, 2048, 512, 32)
        Dh = D // H
        return {'x': _w((lambda *s: _rng.normal(s) * 0.05)(B, S, D)), 'wqkv': _w((lambda *s: _rng.normal(s) * 0.4)(D, 3 * D)), 'w_phi': _w((lambda *s: _rng.normal(s) * 0.4)(H, Dh, Dh) * Dh ** (-0.5)), 'wo': _w((lambda *s: _rng.normal(s) * 0.05)(D, D))}
    _A_in = _A_setup()

    def _B_setup():
        B, S, D, F = (1, 2048, 512, 1792)
        return {'x': _w((lambda *s: _rng.normal(s) * 0.05)(B, S, D)), 'w_gate': _w((lambda *s: _rng.normal(s) * 0.05)(D, F)), 'w_up': _w((lambda *s: _rng.normal(s) * 0.05)(D, F)), 'w_down': _w((lambda *s: _rng.normal(s) * 0.05)(F, D))}
    _B_in = _B_setup()
    return {'A_x': _A_in['x'], 'A_wqkv': _A_in['wqkv'], 'A_w_phi': _A_in['w_phi'], 'A_wo': _A_in['wo'], 'B_x': _B_in['x'], 'B_w_gate': _B_in['w_gate'], 'B_w_up': _B_in['w_up'], 'B_w_down': _B_in['w_down'], 'c': _w((lambda *s: _rng.normal(s) * 0.05)(1, 512) * 8.0), 'w_mod': _w((lambda *s: _rng.normal(s) * 0.05)(512, 6 * 512) * 512 ** (-0.5) * 8.0)}

def reference(A_x, A_wqkv, A_w_phi, A_wo, B_x, B_w_gate, B_w_up, B_w_down, c, w_mod):

    def _A_ref(x, wqkv, w_phi, wo):
        B, S, D = x.shape
        H = 32
        Dh = D // H
        qkv = (lambda x, *d: x.transpose(*d))((x @ wqkv).reshape(B, S, 3, H, Dh), 2, 0, 3, 1, 4)
        q, k, v = (qkv[0], qkv[1], qkv[2])
        pq = jnp.einsum('bhsd,hdf->bhsf', q, w_phi)
        pk = jnp.einsum('bhsd,hdf->bhsf', k, w_phi)
        phi_q = jnp.concatenate([_softmax(pq, axis=-1), _softmax(-pq, axis=-1)], axis=-1)
        phi_k = jnp.concatenate([_softmax(pk, axis=-1), _softmax(-pk, axis=-1)], axis=-1)
        kv = jnp.einsum('bhsf,bhsd->bhfd', phi_k, v)
        z = jnp.einsum('bhsf->bhf', phi_k)
        num = jnp.einsum('bhqf,bhfd->bhqd', phi_q, kv)
        den = jnp.einsum('bhqf,bhf->bhq', phi_q, z)[..., None] + 1e-06
        o = num / den
        return (lambda x, *d: x.transpose(*d))(o, 0, 2, 1, 3).reshape(B, S, D) @ wo

    def _B_ref(x, w_gate, w_up, w_down):
        return _gelu(x @ w_gate) * (x @ w_up) @ w_down
    x = A_x
    mod = (_silu(c) @ w_mod).reshape(c.shape[0], 6, 1, -1)
    sa, ca, ga, sb, cb, gb = (mod[:, 0].copy(), mod[:, 1].copy(), mod[:, 2].copy(), mod[:, 3].copy(), mod[:, 4].copy(), mod[:, 5].copy())
    h = _layernorm(x, axis=-1) * (1 + ca) + sa
    x = x + ga * _A_ref(h, A_wqkv, A_w_phi, A_wo)
    h = _layernorm(x, axis=-1) * (1 + cb) + sb
    x = x + gb * _B_ref(h, B_w_gate, B_w_up, B_w_down)
    return x
```

```python
import jax
import jax.numpy as jnp
import numpy as np
import jax.experimental.pallas as pl
import jax.experimental.pallas.tpu as pltpu

S, D, H, DH, F = 2048, 512, 32, 16, 1792
T = 256
NT = S // T
FC = 256
NB = D // 128

f32 = jnp.float32
bf16 = jnp.bfloat16
NN = (((1,), (0,)), ((), ()))
NTr = (((1,), (1,)), ((), ()))
TN = (((0,), (0,)), ((), ()))


def _dot(a, b, dims=NN):
    return jax.lax.dot_general(a, b, dims, preferred_element_type=f32)


def _ln(x):
    m = jnp.mean(x, axis=-1, keepdims=True)
    xc = x - m
    v = jnp.mean(xc * xc, axis=-1, keepdims=True)
    return xc * jax.lax.rsqrt(v + 1e-5)


def _gelu(x):
    c0 = float(np.sqrt(2.0 / np.pi))
    inner = x * (c0 + (c0 * 0.044715) * (x * x))
    hx = 0.5 * x
    return hx + hx * jnp.tanh(inner)


def _feat(p):
    p3 = p.reshape(DH, 8, p.shape[-1])
    ep = jnp.exp(p3 - jnp.max(p3, axis=0, keepdims=True))
    en = jnp.exp(jnp.min(p3, axis=0, keepdims=True) - p3)
    rp = 1.0 / jnp.sum(ep, axis=0, keepdims=True)
    rn = 1.0 / jnp.sum(en, axis=0, keepdims=True)
    return ep, en, rp, rn


def _kernel(x_hbm, wqkv_hbm, wphi_hbm, wo_hbm, wg_hbm, wu_hbm, wd_hbm, c_hbm, wmod_hbm,
            o_hbm,
            x_v, wqkv_v, wo_v, wg_v, wu_v, wd_v, wmod_v, wqk_t, pq_s, kv_s, z_s, kvt_s, o_v, x1_s, h_s, c_ref, wphi_ref,
            xsem, wsem, osem):
    def xcopy(i):
        return pltpu.make_async_copy(x_hbm.at[pl.ds(i * T, T)], x_v.at[pl.ds(i * T, T)], xsem.at[i])

    def ocopy(i):
        return pltpu.make_async_copy(o_v.at[pl.ds(i * T, T)], o_hbm.at[pl.ds(i * T, T)], osem.at[i])

    def cols(src, dst, j, n, k):
        return pltpu.make_async_copy(src.at[:, pl.ds(j * D, n * D)], dst.at[:, pl.ds(j * D, n * D)], wsem.at[k])

    cp_q, cp_k, cp_v = (cols(wqkv_hbm, wqkv_v, j, 1, 9 + j) for j in range(3))
    cp_m0 = cols(wmod_hbm, wmod_v, 0, 2, 1)
    cp_m1 = cols(wmod_hbm, wmod_v, 2, 4, 2)
    cp_o = pltpu.make_async_copy(wo_hbm, wo_v, wsem.at[3])
    cp_g = pltpu.make_async_copy(wg_hbm, wg_v, wsem.at[4])
    cp_u = pltpu.make_async_copy(wu_hbm, wu_v, wsem.at[5])
    cp_d = pltpu.make_async_copy(wd_hbm, wd_v, wsem.at[6])
    cp_c = pltpu.make_async_copy(c_hbm, c_ref, wsem.at[0])
    cp_p = pltpu.make_async_copy(wphi_hbm, wphi_ref, wsem.at[7])

    for cp in (cp_c, cp_p, cp_m0, xcopy(0), cp_k):
        cp.start()
    kv_s[...] = jnp.zeros_like(kv_s)
    z_s[...] = jnp.zeros_like(z_s)

    def iota(shape, d):
        return jax.lax.broadcasted_iota(jnp.int32, shape, d)

    r1 = iota((D, H), 0)
    sel = ((r1 // 128) * 8 + r1 % 8 == iota((D, H), 1)).astype(bf16)
    fmask = (iota((D, 256), 0) % 128) // 8 == iota((D, 256), 1) % DH
    pick = (iota((256, 128), 0) // DH == iota((256, 128), 1) % DH).astype(bf16)
    pmask = iota((D, 128), 0) % 8 == iota((D, 128), 1) // DH
    cp_p.wait()
    t = jnp.where(fmask, _dot(sel, wphi_ref[...], NTr), 0.0).astype(bf16)
    pm = jnp.where(pmask, _dot(t, pick), 0.0).astype(bf16)
    r2 = iota((128, 128), 0)
    c2 = iota((128, 128), 1)

    cp_c.wait()
    cv = c_ref[...].astype(f32)
    sc = jnp.broadcast_to(cv * jax.nn.sigmoid(cv), (16, D)).astype(bf16)
    cp_m0.wait()
    for cp in (cp_v, cp_q, xcopy(1)):
        cp.start()
    mod0 = _dot(sc, wmod_v[:, pl.ds(0, 2 * D)])
    sa = mod0[0:1, :D]
    ca1 = 1.0 + mod0[0:1, D:]

    def norm1(i):
        rows = pl.ds(pl.multiple_of(i * T, T), T)
        h_s[...] = (_ln(x_v[rows, :].astype(f32)) * ca1 + sa).astype(bf16)

    xcopy(0).wait()
    norm1(0)
    for j, cp in ((1, cp_k), (2, cp_v), (0, cp_q)):
        cp.wait()
        for b in range(NB):
            w = wqkv_v[:, pl.ds(j * D + b * 128, 128)]
            wt = w.T if j == 2 else _dot(pm[b * 128:(b + 1) * 128], w, NTr).astype(bf16)
            wqk_t[pl.ds(j * D + b * 128, 128), :] = wt
    for i in range(2, NT):
        xcopy(i).start()

    def attn_stats(i, last):
        h = h_s[...]
        pk = _dot(wqk_t[pl.ds(D, D), :], h, NTr)
        vt = _dot(wqk_t[pl.ds(2 * D, D), :], h, NTr).astype(bf16)
        if not last:
            norm1(i + 1)
        if not last:
            pq_s[i] = _dot(wqk_t[pl.ds(0, D), :], h, NTr)
        for b in range(NB):
            ep, en, rp, rn = _feat(pk[b * 128:(b + 1) * 128])
            phi = jnp.concatenate([(ep * rp).reshape(128, T), (en * rn).reshape(128, T)], axis=0)
            zs = phi[:, :128]
            for t in range(1, T // 128):
                zs = zs + phi[:, t * 128:(t + 1) * 128]
            z_s[b] += zs
            lo = iota((DH, 8, T), 1) < 4
            pp = ep * rp
            pn = pltpu.roll(en * rn, 4, 1)
            for k, ph in enumerate((jnp.where(lo, pp, pn), jnp.where(lo, pn, pp))):
                r0 = b * 128 + k * 64
                kv_s[b, pl.ds(k * 64, 64), :] += _dot(vt[r0:r0 + 64], ph.reshape(128, T).astype(bf16), NTr)

    def phase1(i, _):
        xcopy(i + 1).wait()

        for k, cp in enumerate((cp_m1, cp_o, cp_g, cp_u, cp_d)):
            pl.when(i == k + 1)(cp.start)
        attn_stats(i, False)
        return None

    jax.lax.fori_loop(0, NT - 1, phase1, None)
    cp_m1.wait()
    cp_o.wait()
    attn_stats(NT - 1, True)
    for b in range(NB):
        kvt_s[b] = jnp.where(c2 % 4 == (r2 // DH) % 4, kv_s[b], 0.0).astype(bf16)
        z_s[b] = jnp.broadcast_to(jnp.sum(z_s[b], axis=-1, keepdims=True), (256, 128))

    mod1 = _dot(sc, wmod_v[:, pl.ds(2 * D, 4 * D)])
    ga = mod1[0:1, :D]
    sb = mod1[0:1, D:2 * D]
    cb1 = 1.0 + mod1[0:1, 2 * D:3 * D]
    gb = mod1[0:1, 3 * D:]

    def attn_steps(i):
        rows = pl.ds(pl.multiple_of(i * T, T), T)
        ots = []
        for b in range(NB):
            ep, en, rp, rn = _feat(pq_s[i, pl.ds(b * 128, 128), :])
            z = jnp.concatenate([z_s[b]] * (T // 128), axis=1).reshape(2 * DH, 8, T)
            den = (jnp.sum(ep * z[:DH], axis=0, keepdims=True) * rp
                   + jnp.sum(en * z[DH:], axis=0, keepdims=True) * rn + 1e-6)
            rd = 1.0 / den
            lo = iota((DH, 8, T), 1) < 4
            pp = ep * (rp * rd)
            pn = pltpu.roll(en * (rn * rd), 4, 1)
            for k, ph in enumerate((jnp.where(lo, pp, pn), jnp.where(lo, pn, pp))):
                ots.append(_dot(kvt_s[b, pl.ds(k * 64, 64), :], ph.reshape(128, T).astype(bf16)))
            yield
        ot = jnp.concatenate(ots, axis=0).astype(bf16)
        x1 = x_v[rows, :].astype(f32) + ga * _dot(ot, wo_v[...], TN)
        yield
        x1_s[...] = x1
        h_s[...] = (_ln(x1) * cb1 + sb).astype(bf16)

    def ffn(i, side=()):
        side = iter(side)
        rows = pl.ds(pl.multiple_of(i * T, T), T)
        h = h_s[...]
        x1 = x1_s[...]
        acc = None
        for j in range(F // FC):
            cols = pl.ds(j * FC, FC)
            a = (_gelu(_dot(h, wg_v[:, cols])) * _dot(h, wu_v[:, cols])).astype(bf16)
            y = _dot(a, wd_v[cols, :])
            acc = y if acc is None else acc + y
            next(side, None)
        o_v[rows, :] = (x1 + gb * acc).astype(o_v.dtype)

    g0 = attn_steps(0)
    next(g0)
    pq_s[NT - 1] = _dot(wqk_t[pl.ds(0, D), :], h_s[...], NTr)
    for _ in g0:
        pass
    for cp in (cp_g, cp_u, cp_d):
        cp.wait()

    def phase2(i, _):
        ffn(i, attn_steps(i + 1))
        ocopy(i).start()
        return None

    jax.lax.fori_loop(0, NT - 1, phase2, None)
    ffn(NT - 1)
    ocopy(NT - 1).start()
    for i in range(NT):
        ocopy(i).wait()


@jax.jit
def pallas_adaLN_cond__linear_kernel_hedgehog__geglu_ffn__prompt_kernel(
    A_x, A_wqkv, A_w_phi, A_wo, B_x, B_w_gate, B_w_up, B_w_down, c, w_mod,
):
    del B_x
    any_spec = pl.BlockSpec(memory_space=pl.ANY)
    out = pl.pallas_call(
        _kernel,
        out_shape=jax.ShapeDtypeStruct((S, D), A_x.dtype),
        in_specs=[any_spec, any_spec, any_spec, any_spec, any_spec, any_spec, any_spec, any_spec, any_spec],
        out_specs=any_spec,
        scratch_shapes=[
            pltpu.VMEM((S, D), bf16),
            pltpu.VMEM((D, 3 * D), bf16),
            pltpu.VMEM((D, D), bf16),
            pltpu.VMEM((D, F), bf16),
            pltpu.VMEM((D, F), bf16),
            pltpu.VMEM((F, D), bf16),
            pltpu.VMEM((D, 6 * D), bf16),
            pltpu.VMEM((3 * D, D), bf16),
            pltpu.VMEM((NT, D, T), f32),
            pltpu.VMEM((NB, 128, 128), f32),
            pltpu.VMEM((NB, 256, 128), f32),
            pltpu.VMEM((NB, 128, 128), bf16),
            pltpu.VMEM((S, D), bf16),
            pltpu.VMEM((T, D), f32),
            pltpu.VMEM((T, D), bf16),
            pltpu.VMEM((1, D), bf16),
            pltpu.VMEM((DH * DH, H), bf16),
            pltpu.SemaphoreType.DMA((NT,)),
            pltpu.SemaphoreType.DMA((12,)),
            pltpu.SemaphoreType.DMA((NT,)),
        ],
        compiler_params=pltpu.CompilerParams(vmem_limit_bytes=100 * 1024 * 1024),
    )(A_x.reshape(S, D), A_wqkv, A_w_phi.transpose(1, 2, 0).reshape(DH * DH, H), A_wo, B_w_gate, B_w_up, B_w_down, c, w_mod)
    return out.reshape(1, S, D)
```
